```python
import os as _os
_os.environ.setdefault("JAX_PLATFORMS", "cpu")
import jax
import jax.numpy as jnp

def _softmax(x, axis=-1):
    return jax.nn.softmax(x, axis=axis)
def _gelu(x):
    return jax.nn.gelu(x, approximate=True)
def _silu(x):
    return jax.nn.silu(x)
def _sigmoid(x):
    return jax.nn.sigmoid(x)
def _layernorm(x, axis=-1, eps=1e-5):
    m = jnp.mean(x, axis=axis, keepdims=True)
    v = jnp.var(x, axis=axis, keepdims=True)
    return (x - m) / jnp.sqrt(v + eps)
def _scatter_add(tgt, idx, src, axis=0):
    return tgt.at[idx].add(src)
def _segment_sum(src, seg, n):
    return jax.ops.segment_sum(src, seg, n)
class _Rng:
    def __init__(self, key):
        self._k = key
    def _next(self):
        self._k, sub = jax.random.split(self._k)
        return sub
    def normal(self, shape):
        return jax.random.normal(self._next(), shape, dtype=jnp.bfloat16)
    def randint(self, lo, hi, shape):
        return jax.random.randint(self._next(), shape, lo, hi, dtype=jnp.int32)
    def uniform(self, shape, lo=0.0, hi=1.0):
        return jax.random.uniform(self._next(), shape, jnp.bfloat16, lo, hi)
    def permutation(self, n):
        return jax.random.permutation(self._next(), n)


kernel_name = 'gated_mix__grouped_kv_mqa__glu_gated_reglu__prompt'

def setup_inputs():
    _rng = _Rng(jax.random.key(int.from_bytes(__import__("os").urandom(4), "little")))
    _w = (lambda a: (lambda t: t.astype(jnp.bfloat16) if jnp.issubdtype(t.dtype, jnp.floating) else t)(jnp.asarray(a)))
    def _A_setup():
        B, S, D, H = 1, 2048, 640, 32
        Dh = D // H
        return {
            "x": _w((lambda *s: _rng.normal(s) * 0.05)(B, S, D)),
            "wq": _w((lambda *s: _rng.normal(s) * 0.2)(D, H * Dh)),
            "wk": _w((lambda *s: _rng.normal(s) * 0.2)(D, Dh)),
            "wv": _w((lambda *s: _rng.normal(s) * 0.05)(D, Dh)),
            "wo": _w((lambda *s: _rng.normal(s) * 0.05)(H * Dh, D)),
        }
    _A_in = _A_setup()

    def _B_setup():
        B, S, D, F = 1, 2048, 640, 1536
        return {
            "x": _w((lambda *s: _rng.normal(s) * 0.05)(B, S, D)),
            "W_gate": _w((lambda *s: _rng.normal(s) * 0.4)(D, F) * (2.0 / D) ** 0.5),
            "W_up": _w((lambda *s: _rng.normal(s) * 0.4)(D, F) * (2.0 / D) ** 0.5),
            "W_down": _w((lambda *s: _rng.normal(s) * 0.4)(F, D) * (1.0 / F) ** 0.5),
        }
    _B_in = _B_setup()

    return {
        "A_x": _A_in["x"],
        "A_wq": _A_in["wq"],
        "A_wk": _A_in["wk"],
        "A_wv": _A_in["wv"],
        "A_wo": _A_in["wo"],
        "B_x": _B_in["x"],
        "B_W_gate": _B_in["W_gate"],
        "B_W_up": _B_in["W_up"],
        "B_W_down": _B_in["W_down"],
        "gate_w": _w((lambda *s: _rng.normal(s) * 0.05)(640) * 16.0),
    }

def reference(A_x, A_wq, A_wk, A_wv, A_wo, B_x, B_W_gate, B_W_up, B_W_down, gate_w):
    def _A_ref(x, wq, wk, wv, wo):
        B, S, D = x.shape
        H = 32
        Dh = D // H
        q = (lambda x, *d: x.transpose(*d))((x @ wq).reshape(B, S, H, Dh), 0, 2, 1, 3)
        k = x @ wk
        v = x @ wv
        scores = jnp.einsum("bhqd,bkd->bhqk", q, k) * (Dh ** -0.5)
        p = _softmax(scores, axis=-1)
        o = jnp.einsum("bhqk,bkd->bhqd", p, v)
        return (lambda x, *d: x.transpose(*d))(o, 0, 2, 1, 3).reshape(B, S, H * Dh) @ wo

    def _B_ref(x, W_gate, W_up, W_down):
        gate = jnp.einsum("bsd,df->bsf", x, W_gate)
        up = jnp.einsum("bsd,df->bsf", x, W_up)
        gate = gate * (lambda x, dt: x.astype(dt))(gate > 0, gate.dtype)
        h = gate * up
        return jnp.einsum("bsf,fd->bsd", h, W_down)

    x = A_x
    g = _sigmoid((x * gate_w).sum(-1, keepdims=True))
    a = _A_ref(x, A_wq, A_wk, A_wv, A_wo)
    b = _B_ref(x, B_W_gate, B_W_up, B_W_down)
    return g * a + (1 - g) * b
```

```python
import jax
import jax.numpy as jnp
from jax import lax
import jax.experimental.pallas as pl
import jax.experimental.pallas.tpu as pltpu

_H = 32
_TQ = 512
_CK = 128
_LOG2E = 1.4426950408889634

_F32 = jnp.float32
_BF16 = jnp.bfloat16


def _dot(a, b):
    return lax.dot_general(a, b, (((1,), (0,)), ((), ())),
                           preferred_element_type=_F32)


def _dot_nt(a, b):
    return lax.dot_general(a, b, (((1,), (1,)), ((), ())),
                           preferred_element_type=_F32)


def _kernel(x_hbm, wq_hbm, wk_hbm, wv_hbm, wo_hbm, wg_hbm, wu_hbm, wd_hbm,
            gw_hbm, out_hbm,
            x_v, wq_v, wk_v, wv_v, wo_v, wg_v, wu_v, wd_v, gw_v,
            wt_v, qt_v, k_v, vt_v, gt_v, gc_v, sa_v, sb_v, ot_v, out_v,
            in_sems, x_sems, out_sems):
    seq, dm = x_v.shape
    dh = dm // _H
    nq = seq // _TQ
    nc = seq // _CK
    qscale = dh ** -0.5 * _LOG2E

    def in_copy(i, src, dst):
        return pltpu.make_async_copy(src, dst, in_sems.at[i])

    def x_copy(i):
        rows = pl.ds(i * _TQ, _TQ)
        return pltpu.make_async_copy(x_hbm.at[rows], x_v.at[rows],
                                     x_sems.at[i])

    def out_copy(i):
        rows = pl.ds(i * _TQ, _TQ)
        return pltpu.make_async_copy(out_v.at[rows], out_hbm.at[rows],
                                     out_sems.at[i])

    early = [in_copy(0, wq_hbm, wq_v), in_copy(1, wk_hbm, wk_v),
             in_copy(2, wv_hbm, wv_v), in_copy(3, gw_hbm, gw_v)]
    late = [in_copy(4, wg_hbm, wg_v), in_copy(5, wu_hbm, wu_v),
            in_copy(6, wd_hbm, wd_v), in_copy(7, wo_hbm, wo_v)]
    for c in early:
        c.start()
    for i in range(nq):
        x_copy(i).start()
    for c in early:
        c.wait()

    wt_v[0:dm, :] = wq_v[...].astype(_F32).T.astype(_BF16)
    gw8 = jnp.broadcast_to(gw_v[...].astype(_F32).reshape(1, dm), (8, dm))
    wt_v[dm:dm + 48, :] = jnp.concatenate(
        [wk_v[...].astype(_F32), wv_v[...].astype(_F32), gw8],
        axis=0).astype(_BF16)

    for i in range(nq):
        x_copy(i).wait()
        if i == nq - 1:
            for c in late:
                c.start()
        rows = slice(i * _TQ, (i + 1) * _TQ)
        p = _dot_nt(wt_v[...], x_v[rows, :])
        qt_v[:, rows] = (p[0:dm] * qscale).astype(_BF16)
        kt = p[dm:dm + dh]
        vt = p[dm + dh:dm + 2 * dh].astype(_BF16).astype(_F32)
        g8 = jax.nn.sigmoid(p[dm + 2 * dh:dm + 2 * dh + 8])
        gt_v[:, rows] = g8
        gc_v[rows, :] = (1.0 - jnp.broadcast_to(g8[0:1], (128, _TQ))).T
        ones = jnp.ones((4, _TQ), _F32)
        vt_v[0, :, rows] = jnp.concatenate([vt, ones], axis=0)
        vt_v[1, :, rows] = jnp.concatenate([ones, vt], axis=0)
        for j in range(4):
            parts = [kt, jnp.zeros((128 - dh - 4 * j, _TQ), _F32)]
            if j:
                parts = [jnp.zeros((4 * j, _TQ), _F32)] + parts
            kj = jnp.concatenate(parts, axis=0).T
            k_v[j, rows, :] = kj[:, 0:32].astype(_BF16)

    sbuf = (sa_v, sb_v)

    def qk(q0, g, j, c, buf, m8):
        r = g * (4 * dh) + 16 * j
        if not isinstance(r, int):
            r = pl.multiple_of(r, 16)
        keys = slice(c * _CK, (c + 1) * _CK)
        s = _dot(k_v[j, keys, :], qt_v[pl.ds(r, 32), pl.ds(q0, _TQ)])
        buf[keys, :] = s
        mc = jnp.max(s.reshape(_CK // 8, 8, _TQ), axis=0)
        return mc if m8 is None else jnp.maximum(m8, mc)

    def pv(j, c, buf, m, o, zero):
        keys = slice(c * _CK, (c + 1) * _CK)
        r = pl.multiple_of(zero + c * _CK, _CK)
        p = jnp.exp2(buf[pl.ds(r, _CK), :] - m).astype(_BF16)
        oc = _dot(vt_v[j % 2, :, keys], p)
        return oc if o is None else o + oc

    m8 = None
    for c in range(nc):
        m8 = qk(0, 0, 0, c, sa_v, m8)

    ng = _H // 4

    def group(it, m8):
        g = it % ng
        q0 = pl.multiple_of((it // ng) * _TQ, _TQ)
        nxt = jnp.minimum(it + 1, nq * ng - 1)
        gn = nxt % ng
        q0n = pl.multiple_of((nxt // ng) * _TQ, _TQ)
        gate = gt_v[0:1, pl.ds(q0, _TQ)]
        zero = (it // (nq * ng)) * _CK
        prev = None
        for j in range(4):
            m = jnp.max(m8, axis=0, keepdims=True)
            m8, o = None, None
            for c in range(nc):
                if j < 3:
                    m8 = qk(q0, g, j + 1, c, sbuf[(j + 1) % 2], m8)
                else:
                    m8 = qk(q0n, gn, 0, c, sbuf[0], m8)
                o = pv(j, c, sbuf[j % 2], m, o, zero)
            lrow = dh if j % 2 == 0 else 0
            o = o * (gate / o[lrow:lrow + 1, :])
            if j % 2 == 0:
                prev = o
            else:
                sub = lax.broadcasted_iota(jnp.int32, (8, _TQ), 0)
                mid = jnp.where(sub < 4, prev[16:24], o[0:8])
                r0 = pl.multiple_of(g * (4 * dh) + (j // 2) * (2 * dh), 8)
                ot_v[pl.ds(r0, 2 * dh), pl.ds(q0, _TQ)] = jnp.concatenate(
                    [prev[0:16], mid, o[8:24]], axis=0)
        return m8

    lax.fori_loop(0, nq * ng, group, m8)

    for c in late:
        c.wait()

    def mix(i, _):
        r0 = pl.multiple_of(i * _TQ, _TQ)
        rows = pl.ds(r0, _TQ)
        xb = x_v[rows, :]
        gate = _dot(xb, wg_v[...])
        up = _dot(xb, wu_v[...])
        h = (jnp.maximum(gate, 0.0) * up).astype(_BF16)
        b = _dot(h, wd_v[...])
        a = _dot(ot_v[:, rows].T.astype(_BF16), wo_v[...])
        gc = gc_v[rows, :]
        gc = jnp.concatenate([gc] * (dm // 128), axis=1)
        out_v[rows, :] = (a + gc * b).astype(out_v.dtype)
        pltpu.make_async_copy(out_v.at[rows], out_hbm.at[rows],
                              out_sems.at[i]).start()

    lax.fori_loop(0, nq, mix, None)
    for i in range(nq):
        out_copy(i).wait()


@jax.jit
def pallas_gated_mix__grouped_kv_mqa__glu_gated_reglu__prompt_kernel(
    A_x: jax.Array,
    A_wq: jax.Array,
    A_wk: jax.Array,
    A_wv: jax.Array,
    A_wo: jax.Array,
    B_x: jax.Array,
    B_W_gate: jax.Array,
    B_W_up: jax.Array,
    B_W_down: jax.Array,
    gate_w: jax.Array,
):
    del B_x
    batch, seq, dm = A_x.shape
    assert batch == 1
    nq = seq // _TQ
    vmem = pltpu.VMEM

    def like(a):
        return vmem(a.shape, a.dtype)

    x = A_x.reshape(seq, dm)
    ins = (x, A_wq, A_wk.T, A_wv.T, A_wo, B_W_gate, B_W_up, B_W_down, gate_w)
    out = pl.pallas_call(
        _kernel,
        out_shape=jax.ShapeDtypeStruct((seq, dm), A_x.dtype),
        in_specs=[pl.BlockSpec(memory_space=pl.ANY)] * len(ins),
        out_specs=pl.BlockSpec(memory_space=pl.ANY),
        scratch_shapes=[
            *[like(a) for a in ins],
            vmem((dm + 48, dm), _BF16),
            vmem((dm, seq), _BF16),
            vmem((4, seq, 32), _BF16),
            vmem((2, 24, seq), _F32),
            vmem((8, seq), _F32),
            vmem((seq, 128), _F32),
            vmem((seq, _TQ), _F32),
            vmem((seq, _TQ), _F32),
            vmem((dm, seq), _F32),
            vmem((seq, dm), A_x.dtype),
            pltpu.SemaphoreType.DMA((8,)),
            pltpu.SemaphoreType.DMA((nq,)),
            pltpu.SemaphoreType.DMA((nq,)),
        ],
        compiler_params=pltpu.CompilerParams(
            vmem_limit_bytes=100 * 1024 * 1024),
        name="gated_mix_mqa_reglu",
    )(*ins)
    return out.reshape(batch, seq, dm)
```

```python
import functools

import jax
import jax.numpy as jnp
from jax import lax
import jax.experimental.pallas as pl
import jax.experimental.pallas.tpu as pltpu


_H = 32
_T = 128
_HT = _T // 2
_PB = 512
_STEPS = 8
_LOG2E = 1.4426950408889634
_SCORE_LIMIT = 40.0
_BALANCE = 64.0
_ZEROS = 32

_TABLES = (5, 2)
_AHEAD = 3
_LAG = 4
_BATCH = 20
_SCORE_LATENCY = 193
_PV_LATENCY = 165
_WAVE_LATENCY = 183
_SEGMENT = 900
_PHASES = (
    (13, -2, 0, 0, 0), (0, 0, -2, 0, 0), (0, 0, 0, 0, 10), (0, 5, 6, 4, 5),
    (7, 0, 0, 0, 0), (0, 0, 0, 0, 5), (0, 3, 0, 7, 0), (0, 0, 0, 3, -3),
    (15, -2, 0, 0, 0), (11, 4, -5, 8, 5), (5, 0, 0, 0, 5), (0, 2, 0, 0, 3),
    (8, 0, 0, 0, 0), (7, -2, -3, 5, 7), (2, -3, 0, 0, 0), (0, 0, 0, 0, 2),
    (3, 1, -6, -8, -5), (0, 0, 5, 0, 0), (3, 3, -6, -8, 5), (7, 11, -3, 1, -6),
    (7, 0, 0, 0, 0), (0, -11, 0, 2, -5), (0, 0, 0, 5, 0), (0, 0, 0, 0, -7),
    (0, 0, 0, 0, 12))

_F32 = jnp.float32
_BF16 = jnp.bfloat16
_U32 = jnp.uint32


def _dot(a, b):
    return lax.dot_general(a, b, (((1,), (0,)), ((), ())),
                           preferred_element_type=_F32)


def _dot_nt(a, b):
    return lax.dot_general(a, b, (((1,), (1,)), ((), ())),
                           preferred_element_type=_F32)


def _pack(v):
    return pltpu.bitcast(v.astype(_BF16), _U32)


def _unpack(v):
    return pltpu.bitcast(v, _BF16)


def _transpose(v):
    return pltpu.bitcast(pltpu.bitcast(v, _U32).T, _F32)


def _al(v, m):
    return v if isinstance(v, int) else pl.multiple_of(v, m)


def _cols(n, count=1):
    return slice(n * _T, (n + count) * _T)


def _cat(parts, axis):
    return jnp.concatenate(list(parts), axis=axis)


def _strassen_lhs(a11, a12, a21, a22):
    return a11 + a22, a21 + a22, a11, a22, a11 + a12, a21 - a11, a12 - a22


def _strassen_rhs(b11, b12, b21, b22):
    return b11 + b22, b11, b12 - b22, b21 - b11, b22, b11 + b12, b21 + b22


_STRASSEN_OUT = (
    ((0, 0, 1), (1, 1, 1)), ((1, 0, 1), (1, 1, -1)), ((0, 1, 1), (1, 1, 1)),
    ((0, 0, 1), (1, 0, 1)), ((0, 0, -1), (0, 1, 1)), ((1, 1, 1),),
    ((0, 0, 1),))

_WINOGRAD = (
    ((), ((0,),)), ((0,), ((None, 0, 0),)), ((0,), ((0,),)), ((0,), ((1,),)),
    ((1,), ((None, 1, 0),)), ((0, 1), ((0,), (None, 1, 2))),
    ((0,), ((None, 0, 2),)))
_WINOGRAD_QUERY = ((0, 0), (1, 0), (0, 4), (1, 4), (1, 6), (0, 6), (1, 2))


def _winograd_keys(a11, a12, a21, a22):
    s1 = a21 + a22
    s2 = s1 - a11
    return a11, a12, s2, a11 - a21, a22, s1, a12 - s2


def _winograd_queries(q1, q2):
    even = (lax.broadcasted_iota(jnp.int32, q1.shape, 0) & 1) == 0
    odd2 = pltpu.roll(q2, 7, 0)
    t1 = q2 - q1
    t2 = odd2 - t1
    return (jnp.where(even, t2, pltpu.roll(odd2 - q2, 1, 0)),
            jnp.where(even, t1, q1 - pltpu.roll(t2, 1, 0)))


def _feeders(a, b):
    return [j for j in range(7) for o in _STRASSEN_OUT[j] if o[:2] == (a, b)]


def _combine(old, sign, y):
    return y if old is None else old + y if sign > 0 else old - y


def _operand(base, i, rows):
    return base + (i // 2) * rows, 2 * (i % 2)


def _rows(**sizes):
    start, total = {}, 0
    for name, size in sizes.items():
        start[name] = total
        total += size
    return start, total


def _layouts(seq, dm, ff):
    pairs = ff // (2 * _T)
    work = _rows(
        wq=dm,
        k=seq // 2,
        p=seq,
        o=_T,
        h=(pairs // 2) * 5 * (_HT // 2),
        gu=2 * _T,
        tmp=_HT,
        acc=2 * _T,
        b=2 * _T,
        pv=24,
        sw=64,
        gc=_T // 4,
        x=2 * _T)
    weights = _rows(
        kv=48,
        x=_PB,
        gu=pairs * 4 * _T,
        down=(pairs // 2) * 4 * _T,
        o=4 * _T,
        rows=(2 + pairs // 2) * _T,
        columns=8 * (pairs + 1))
    return work, weights


def _phase(kind, time):
    segment = min(max(int(time // _SEGMENT), 0), len(_PHASES) - 1)
    return _PHASES[segment][kind]


class _Timeline:
    def __init__(self, phased):
        self.events = []
        self.phased = phased

    def at(self, time, fn, *args):
        self.events.append((time, len(self.events), fn, args))

    def load_at(self, time, fn, *args, after=-1e9):
        phase = _phase(0, time) if self.phased else 0
        self.at(max((time - phase) // _BATCH * _BATCH + phase, after), fn,
                *args)

    def run(self):
        for _, _, fn, args in sorted(self.events, key=lambda e: e[:2]):
            fn(*args)


def _kernel(x_hbm, wq_hbm, wk_hbm, wv_hbm, wo_hbm, wg_hbm, wu_hbm, wd_hbm,
            gw_hbm, out_hbm,
            x_v, wq_v, wo_v, wd_v, wgu_v, out_v, mem, wp, qt_v, qf_v, kb0_v,
            kb1_v, vt_v, gt_v, ot_v, wk_v, wv_v, gw_v,
            zero_s, in_sems, x_sems, out_sem):
    seq, dm = x_v.shape
    ff = wd_v.shape[0]
    dh = dm // _H
    nt = seq // _T
    pairs = ff // (2 * _T)
    nk = pairs // 2
    (lay, _), (wlay, _) = _layouts(seq, dm, ff)

    def in_copy(i, src, dst):
        return pltpu.make_async_copy(src, dst, in_sems.at[i])

    def x_copy(i):
        rows = pl.ds(_al(i * _PB, _PB), _PB)
        return pltpu.make_async_copy(x_hbm.at[rows], x_v.at[rows],
                                     x_sems.at[i])

    def out_copy(t):
        rows = pl.ds(_al(t * _T, _T), _T)
        return pltpu.make_async_copy(out_v.at[rows], out_hbm.at[rows],
                                     out_sem)

    def zeros():
        count = [0]

        def zero():
            count[0] += 1
            return zero_s[count[0] % _ZEROS]
        return zero

    tables = (kb0_v, kb1_v)
    vpu = [i * (_PB // 16) + 2 * e for i in range(4)
           for e in range(_TABLES[i // 2])]
    mxu = [g for g in range(seq // 16) if g - g % 2 not in vpu]
    chunks = [mxu[len(mxu) * c // nt:len(mxu) * (c + 1) // nt]
              for c in range(nt)]
    ahead = vpu[:_AHEAD]
    groups = [(u, e) for u in range(_STEPS) for e in vpu][_AHEAD:]
    groups += [(_STEPS, e) for e in ahead]
    stages = [stage[1:] for stage in sorted(
        (7 * n + 2 * i, n % 4, *group, i)
        for n, group in enumerate(groups) for i in range(7))]

    def key_home(i, d):
        row = 4 * dh * (i % 4) + 8 * d
        return slice(row, row + 8), _cols(2 * (i < 4), 2)

    def p_row(u, g):
        return lay["p"] + (u % 2) * (seq // 2) + 8 * g

    def score_stage(tile, u, e, i, sums, z):
        block, e0 = divmod(e, _PB // 16)
        k = tables[block // 2].at[
            (block % 2) * _TABLES[block // 2] + e0 // 2 + z]
        q = qf_v.at[tile + z]
        odd, col = _WINOGRAD_QUERY[i]
        acc = [None, None]
        for d in range(dh // 2):
            kd = k[key_home(i, d)]
            kd = _cat([kd[:, _cols(0)], kd[:, _cols(1)]], 0)
            r = dh * u + 2 * d + odd
            for j in range(2):
                acc[j] = _combine(acc[j], 1, kd * q[r:r + 1, _cols(col + j)])
        y = _cat(acc, 1)
        olds = [sums[j] for j in _WINOGRAD[i][0]] or [None]
        for out, old in zip(_WINOGRAD[i][1], olds):
            v = _combine(old, 1, y)
            if out[0] is None:
                row = p_row(u, e + out[1]) + z
                mem[pl.ds(_al(row, 8), 8), _cols(out[2], 2)] = _pack(
                    jnp.exp2(v))
            else:
                yield out[0], v

    def note_rows(panel, r, quad):
        v = _cat([quad[0][:, _cols(0)], quad[2][:, _cols(0)]], 1)
        row = wlay["rows"] + r // 2 + panel * _T
        wp[pl.ds(_al(row, 8), 8), _cols(0, 2)] = _pack(v * v)

    def note_columns(panel, quad):
        top, bottom = _cat(quad[0:2], 1), _cat(quad[2:4], 1)
        sq = top * top + bottom * bottom
        row = wlay["columns"] + panel * 8
        wp[pl.ds(_al(row, 8), 8), :] = pltpu.bitcast(sq[0:8] + sq[8:16], _U32)

    def balanced():
        rows = wp.at[pl.ds(_al(wlay["rows"] + zero_s[0], 8), (2 + nk) * _T)]
        sums = [[_dot_nt(jnp.ones((16, _T), _BF16),
                         _unpack(rows[:, _cols(n)]))[0:1] for n in range(2)]]
        for panel in range(pairs + 1):
            row = wlay["columns"] + panel * 8
            v = jnp.sum(pltpu.bitcast(wp[row:row + 8, :], _F32), 0,
                        keepdims=True)
            sums.append([v[:, _cols(0, 2)], v[:, _cols(2, 2)]])
        a, b = (_cat(side, 1) for side in zip(*sums))
        return jnp.min(jnp.minimum(_BALANCE * a - b, _BALANCE * b - a)) >= 0.0

    def prepare_gate_up(j, n, r):
        w = wgu_v.at[j]

        def block(row, half):
            return w[row + r:row + r + 16, _cols(n + pairs * half, 2)]

        quad = [block(row, half).astype(_F32)
                for row in (0, 2 * _T) for half in range(2)]
        if n == 0:
            note_rows(j, r, quad)
        if r == 0:
            note_columns(n + j, quad)
        outs = [(*_operand(0, i, _T), v)
                for i, v in enumerate(_strassen_rhs(*quad))]
        if r < _T:
            outs += [(3 * _T + _HT * half, 2, block(4 * _T, half))
                     for half in range(2)]
        for row, col, v in outs:
            row += wlay["gu"] + n * 4 * _T + r // 2 + j * 4 * _T
            wp[pl.ds(_al(row, 8), 8), _cols(col, 2)] = _pack(v)

    def prepare_down(r):
        kk, sub = divmod(r, 2 * _T)
        base = wlay["down"] + kk * 4 * _T + sub // 2
        quad = [wd_v[k0 + r:k0 + r + 16, _cols(c, 2)].astype(_F32)
                for k0 in (0, ff // 2) for c in (0, 2)]
        note_rows(2 + kk, sub, quad)
        if r == 0:
            note_columns(pairs, quad)
        for i, v in enumerate(_strassen_rhs(*quad)):
            row, col = _operand(base, i, _T)
            wp[row:row + 8, _cols(col, 2)] = _pack(v)
        for half in range(2):
            row, k0 = base + 3 * _T, half * (ff // 2) + r
            wp[row:row + 8, _cols(2 + half)] = _pack(
                wd_v[k0:k0 + 16, _cols(4)])

    def prepare_out(packed):
        for n in range(5):
            row = wlay["o"] + 2 * _T * (n // 4)
            wp[row:row + 2 * _T, _cols(n % 4)] = packed(slice(0, 4 * _T),
                                                        _cols(n))
        row = wlay["o"] + 2 * _T
        wp[row:row + _HT, _cols(1, 3)] = packed(_cols(4), _cols(0, 3))
        wp[row + _HT:row + _T, _cols(1, 2)] = packed(_cols(4), _cols(3, 2))

    def stage_x(t, r, c):
        tile = x_v.at[pl.ds(_al(t * _T, _T), _T)]

        def block(half, col):
            return tile[_HT * half + r:_HT * half + r + 16, _cols(col)]

        outs = list(enumerate(_strassen_lhs(*(
            block(half, c + col).astype(_F32)
            for half in range(2) for col in (0, 2)))))
        for m, v in (*outs, (7, block(c, 4))):
            row, col = _operand(lay["x"] + r // 2, m, _HT // 2)
            row += (t & 1) * _T
            mem[pl.ds(_al(row, 8), 8), _cols(col + c)] = _pack(v)

    def gate_row(t):
        return gt_v[0:1, pl.ds(_al(t * _T, _T), _T)]

    def one_minus_gate(t):
        return jnp.broadcast_to(1.0 - gate_row(t), (_T, _T)).T

    small = [in_copy(0, wk_hbm, wk_v), in_copy(1, wv_hbm, wv_v),
             in_copy(2, gw_hbm, gw_v)]
    wq_copy = in_copy(3, wq_hbm, wq_v)
    gate_up_copies = [in_copy(4, wg_hbm, wgu_v.at[0]),
                      in_copy(5, wu_hbm, wgu_v.at[1])]
    wd_copy = in_copy(6, wd_hbm, wd_v)
    wo_copy = in_copy(7, wo_hbm, wo_v)
    for copy in (wq_copy, *small, x_copy(0)):
        copy.start()
    for i in range(_ZEROS):
        zero_s[i] = 0
    ot_v[...] = jnp.zeros(ot_v.shape, _F32)
    mem[lay["b"]:lay["pv"], :] = jnp.zeros((2 * _T, 4 * _T), _U32)
    prepare_out(lambda r, c: jnp.zeros(
        ((r.stop - r.start) // 2, c.stop - c.start), _U32))
    wq_copy.wait()

    def put_wide(dst, row, value):
        rows = value.shape[0]
        dst[row:row + rows, :] = value[:, _cols(0, 4)]
        dst[row + rows:row + 2 * rows, _cols(0)] = value[:, _cols(4)]

    put_wide(mem, lay["wq"], _pack(_transpose(wq_v[...].astype(_F32))))
    x_copy(1).start()
    gate_up_copies[0].start()
    for copy in small:
        copy.wait()
    gw8 = jnp.broadcast_to(gw_v[...].astype(_F32).reshape(1, dm), (8, dm))
    put_wide(wp, wlay["kv"], _pack(_cat(
        [wk_v[...].astype(_F32), wv_v[...].astype(_F32), gw8], 0)))

    def project(second, j, bounds):
        i = j + 2 * second
        x_copy(i).wait()

        @pl.when(j == 0)
        def _():
            if second:
                gate_up_copies[0].wait()
                wd_copy.start()
            else:
                x_copy(2).start()

        @pl.when(j == 1)
        def _():
            if second:
                gate_up_copies[1].wait()
            else:
                x_copy(3).start()
                gate_up_copies[1].start()

        line, live, zero = _Timeline(False), {}, zeros()
        q_sq, k_sq, v_abs = bounds
        rows = pl.ds(_al(i * _PB, _PB), _PB)

        def x_home(tile):
            t, k = divmod(tile, 5)
            return wlay["x"] + _HT * t + (_PB // 2) * (k // 4), _cols(k % 4)

        xb = x_v[rows, :]
        for tile in range(20):
            row, cols = x_home(tile)
            wp[row:row + _HT, cols] = _pack(xb[_cols(tile // 5),
                                               _cols(tile % 5)])
        p = _dot_nt(_unpack(_cat([wp[0:24, :], wp[24:48, _cols(0)]], 1)), xb)
        kt = p[0:dh]
        vt = p[dh:2 * dh].astype(_BF16).astype(_F32)
        k_sq = jnp.maximum(k_sq, jnp.sum(kt * kt, 0, keepdims=True))
        v_abs = jnp.maximum(v_abs, jnp.max(jnp.abs(vt), 0, keepdims=True))
        gt_v[:, rows] = jax.nn.sigmoid(p[2 * dh:2 * dh + 8])
        ones = jnp.ones((4, _PB), _F32)
        vt_v[0, :, rows] = _cat([vt, ones], 0)
        vt_v[1, :, rows] = _cat([ones, vt], 0)
        vt_v[2, :, 0:_PB] = _cat([kt, jnp.zeros_like(ones)], 0)

        def k_tile(t):
            kt = vt_v[2 + zero(), :, _cols(t)]
            return _cat([kt, jnp.zeros((_T - 24, _T), _F32)], 0).T

        n = _TABLES[second]
        keys = _cat((k_tile(t) for t in range(pl.cdiv(32 * n, _T))), 0)
        for d in range(dh // 2):
            wide = [jnp.broadcast_to(keys[0:32 * n, lane:lane + 1],
                                     (32 * n, _T))
                    for lane in (2 * d, 2 * d + 1)]
            for e in range(n):
                for m, v in enumerate(_winograd_keys(*(
                        w[32 * e + r:32 * e + r + 16]
                        for r in (0, 16) for w in wide))):
                    tables[second][(j * n + e, *key_home(m, d))] = _cat(
                        [v[0:8], v[8:16]], 1)

        def put_k(t):
            packed = _pack(k_tile(t))
            row = lay["k"] + i * (_PB // 2) + t * _HT
            mem[pl.ds(_al(row, 8), _HT), :] = _cat(
                [pltpu.roll(packed, 4 * v, 1) if v else packed
                 for v in range(4)], 1)

        per_group = 4 * dh // 16
        pieces = [(half, m + 2 * n, sub) for half in range(2)
                  for m in range(2) for sub in range(per_group)
                  for n in range(2)]
        per_part = len(pieces) // 4

        def lhs_load(r):
            half, m, sub = pieces[r]
            row = lay["wq"] + 8 * ((4 * half + m) * per_group + sub) + zero()
            live["lhs", r] = _cat(
                [mem[pl.ds(_al(row, 8), 8), :],
                 mem[pl.ds(_al(row + dm // 2, 8), 8), _cols(0)]], 1)

        def x_load(n, wave):
            z = zero()
            for tile in range(4 * wave, 4 * wave + 4):
                row, cols = x_home(tile)
                live["x", n, tile] = wp[pl.ds(_al(row + z, 8), _HT), cols]

        def part(n):
            lhs = _cat((live.pop(("lhs", per_part * n + r))
                        for r in range(per_part)), 0)
            rhs = _cat((_cat((live.pop(("x", n, 5 * t + k)) for k in range(5)),
                             1) for t in range(4)), 0)
            live["y", n] = _dot_nt(_unpack(lhs), _unpack(rhs))

        def done(w, r):
            at = 16 * (r % per_part)
            q = live["y", r // per_part][at:at + 16, _cols(w)] * (
                dh ** -0.5 * _LOG2E)
            half, m, sub = pieces[r]
            tile, row = 4 * i + w, 4 * dh * half + 16 * sub
            qf_v[tile, row:row + 16, _cols(m)] = q
            qt_v[tile, row // 2:row // 2 + 8, _cols(m)] = _pack(q)
            mem[pl.ds(_al(lay["pv"] + zero(), 8), 8), _cols(m)] = _pack(q)
            if m < 2:
                live["q1"] = q
                return
            q1 = live.pop("q1")
            for at in (0, 8):
                for n, v in enumerate(_winograd_queries(q1[at:at + 8],
                                                        q[at:at + 8])):
                    qf_v[tile, row + at:row + at + 8, _cols(2 + m + 2 * n)] = v
            sq = jnp.maximum(q * q, q1 * q1)
            live["sq", w] = _combine(live["sq", w] if sub else None, 1,
                                     sq[0:8] + sq[8:16])
            if sub == per_group - 1:
                live["q_sq"] = jnp.maximum(
                    live.get("q_sq", q_sq),
                    jnp.sum(live["sq", w], 0, keepdims=True))

        span = 16 * per_part
        early = 4 * span
        for n in range(4):
            time = 240 + 5 * span * n
            for r in range(per_part):
                line.load_at(time + 16 * r, lhs_load, per_part * n + r)
                for w in range(4):
                    line.at(time + span * (w + 1) + 16 * r + 185, done, w,
                            per_part * n + r)
            for wave in range(5):
                line.at(time + span * wave - 30 - early, x_load, n, wave)
            line.at(time + span, part, n)
        for t in range(4):
            line.at(2600 + 300 * t, put_k, t)
        if second:
            work = [(n, r) for n in range(0, pairs, 2)
                    for r in range(0, 2 * _T, 16)]
            for m, (n, r) in enumerate(work):
                line.at(250 + 3200 * m / len(work) - early, prepare_gate_up,
                        j, n, r)
        line.run()
        return live["q_sq"], k_sq, v_abs

    bounds = tuple(jnp.zeros((1, n), _F32) for n in (_T, _PB, _PB))
    for second in range(2):
        bounds = lax.fori_loop(0, 2, functools.partial(project, second),
                               bounds)
    wd_copy.wait()
    wo_copy.start()
    for r in range(0, ff // 2, 16):
        prepare_down(r)
    q_sq, k_sq, v_max = (jnp.max(b) for b in bounds)
    fast_ok = ((q_sq * k_sq <= _SCORE_LIMIT ** 2)
               & (v_max <= 2.0 ** 60) & (v_max >= 2.0 ** -50)
               & balanced())
    for r in range(0, _HT, 16):
        for c in range(2):
            stage_x(0, r, c)
    for e in ahead:
        sums = {}
        for i in range(7):
            sums.update(list(score_stage(0, 0, e, i, sums, 0)))

    def q_window(t, half, j):
        return _unpack(qt_v[t, pl.ds(_al(2 * dh * half + 8 * j, 8), 16), :])

    def normalise(o, odd, t):
        lrow = 0 if odd else dh
        total = o[lrow:lrow + 1, :]
        r = pltpu.reciprocal(total, approx=True)
        r = r * (2.0 - total * r)
        return o * (_cat([gate_row(t)] * 4, 1) * r)

    def low_rows_from(a, b):
        sub = lax.broadcasted_iota(jnp.int32, a.shape, 0)
        return jnp.where(sub < 4, a, b)

    def o_tile(lo, hi):
        parts = []
        for grp in range(_H // 4):
            half, m = divmod(grp, 4)
            a, b = max(lo, 4 * dh * grp), min(hi, 4 * dh * (grp + 1))
            if a < b:
                shift = 4 * dh * (half - grp)
                parts.append(ot_v[a + shift:b + shift, _cols(m)])
        return _transpose(_cat(parts, 0))

    def fast_tile(t, carry):
        line, live, zero = _Timeline(True), {}, zeros()
        following = (t + 1) & (nt - 1)
        owner = {p_row(0, e + j): 0 for e in ahead for j in range(2)}
        newest = {}

        def touch(row, rows, cols, write):
            for r in range(row, row + rows, 8):
                for c in range(cols.start, cols.stop, _T):
                    wrote, read = newest.get((r, c), ((-1,), (-1,)))
                    now = live["now"]
                    assert wrote <= now and (read <= now or not write)
                    newest[r, c] = (now, read) if write else (
                        wrote, max(read, now))

        def load(row, rows, cols):
            if row >= lay["x"]:
                row += (t & 1) * _T + zero()
                return mem[pl.ds(_al(row, 8), rows), cols]
            touch(row, rows, cols, False)
            return mem[row:row + rows, cols]

        def store(row, cols, value):
            touch(row, value.shape[0], cols, True)
            mem[row:row + value.shape[0], cols] = value

        def get(row, cols, rows=16):
            return pltpu.bitcast(load(row, rows, cols), _F32)

        def put(row, cols, value):
            store(row, cols, pltpu.bitcast(value, _U32))

        def q_load(u, c):
            live["q", u, c] = q_window(t + zero(), u // 4, u % 4)

        def k_load(u, g):
            row = lay["k"] + 8 * g
            live["k", u, g] = mem[row:row + 8, _cols(u % 4)]

        def qk(u, c):
            k = _cat((live.pop(("k", u, g)) for g in chunks[c]), 0)
            live["s", u, c] = _dot(_unpack(k)[:, :32], live.pop(("q", u, c)))

        def p_store(u, c, i):
            row = p_row(u, chunks[c][i])
            mem[row:row + 8, :] = _pack(
                jnp.exp2(live["s", u, c][16 * i:16 * i + 16]))
            owner[row] = u

        def sums_fetch(slot, u, e, i):
            assert i == 0 or live.pop(("slot", slot)) == (u, e, i - 1)
            row = lay["sw"] + 16 * slot
            live["sums", u, e, i] = {
                j: pltpu.bitcast(mem[row:row + 16, _cols(2 * j, 2)], _F32)
                for j in _WINOGRAD[i][0]}

        def scores(slot, u, e, i):
            z = zero()
            row = lay["sw"] + 16 * slot
            for j, v in score_stage(t if u < _STEPS else following, u % _STEPS,
                                    e, i, live.pop(("sums", u, e, i)), z):
                mem[pl.ds(_al(row + z, 8), 16), _cols(2 * j, 2)] = (
                    pltpu.bitcast(v, _U32))
            live["slot", slot] = (u, e, i)
            if i == 6:
                owner.update({p_row(u, e): u, p_row(u, e + 1): u})

        pv_order = {}

        def p_load(u, c, part):
            row = p_row(u, 8 * pv_order[u][c] + 2 * part)
            assert owner[row] == owner[row + 8] == u
            live["p", u, c, part] = mem[pl.ds(_al(row + zero(), 8), 16), :]

        def pv(u, c):
            p = _cat((live.pop(("p", u, c, part)) for part in range(4)), 0)
            live["o", u, c] = _dot(vt_v[u % 2, :, _cols(pv_order[u][c])],
                                   _unpack(p))

        def o_fetch(u, c, r):
            live["now"] = (u, c, 0)
            live["old", u, c, r] = get(lay["pv"] + r, _cols(0, 4), 8)

        def o_done(u, c, r):
            live["now"] = (u, c, 1)
            o = _combine(live.pop(("old", u, c, r), None), 1,
                         live["o", u, c][r:r + 8])
            if c < nt - 1:
                return put(lay["pv"] + r, _cols(0, 4), o)
            live["sum", r] = o
            if r < 16:
                return
            o = normalise(_cat((live.pop(("sum", i)) for i in (0, 8, 16)), 0),
                          u % 2, t + zero())
            row = 2 * dh * (u // 2) + 16 * (u % 2)
            if u % 2:
                mid = ot_v[pl.ds(_al(row + zero(), 8), 8), :]
                o = _cat([low_rows_from(mid, o[0:8]), o[8:24]], 0)
            ot_v[row:row + 24, :] = o

        def span(row, n, cols):
            return [[(row + 8 * r, cols)] for r in range(n)]

        def weight(row, rows, cols):
            return lambda: _unpack(wp[row:row + rows, cols])

        def h_operand(n, i):
            return _operand(lay["h"] + (n // 2) * 5 * (_HT // 2), i, _HT // 2)

        def gate_up(j, i, r):
            outs = []
            for a, b, sign in _STRASSEN_OUT[i]:
                row = lay["gu"] + _T * j + _HT * a + 16 * r
                cols = _cols(2 * b, 2)
                outs.append((row, cols, sign, get(row, cols)
                             if i > _feeders(a, b)[0] else None))
            y = yield
            for row, cols, sign, old in outs:
                put(row, cols, _combine(old, sign, y))

        def hidden(n, r):
            row = lay["gu"] + _HT * (r % 2) + 16 * (r // 2)
            old = _cat((get(row + _T * j, _cols(2 * b + n % 2))
                        for b in range(2) for j in range(2)), 1)
            y = (yield) + old
            h = [jnp.maximum(y[:, _cols(i)], 0.0) * y[:, _cols(i + 1)]
                 for i in (0, 2)]
            if r % 2 == 0:
                live["h"] = h
                return
            top = live.pop("h")
            for i, v in enumerate((*_strassen_lhs(*top, *h), top[1], h[0])):
                row, col = h_operand(n, i)
                store(row + 8 * (r // 2), _cols(col + n % 2), _pack(v))

        def project_out(n, r):
            row, cols = lay["b"] + _T * (n // 4) + 16 * r, _cols(n % 4)
            old = get(row, cols)
            put(row, cols, (yield) + old)

        def emit(n, count, r):
            old = get(lay["b"] + _T * (n // 4) + 16 * r, _cols(0, count))
            rows = pl.ds(_al(jnp.maximum(t - 1, 0) * _T + 16 * r, 16), 16)
            out_v[rows, _cols(n, count)] = ((yield) + old).astype(out_v.dtype)

        def stage_gate():
            gc = one_minus_gate(t)
            for r in range(0, _T, 16):
                live["now"] = (-1,)
                put(lay["gc"] + r % 32, _cols(r // 32), gc[r:r + 16])
                yield

        def gate_rows(row):
            return get(lay["gc"] + row % 32, _cols(row // 32))

        def down(i, kk, r):
            row, cols = lay["tmp"] + 16 * r, _cols(0, 2)
            part = get(row, cols) if kk else None
            if kk < nk - 1:
                return put(row, cols, _combine(part, 1, (yield)))
            outs = []
            for a, b, sign in _STRASSEN_OUT[i]:
                row, cols = _HT * a + 16 * r, _cols(2 * b, 2)
                last = i == _feeders(a, b)[-1]
                outs.append((row, cols, sign, gate_rows(row) if last else None,
                             get(lay["acc"] + row, cols)
                             if i > _feeders(a, b)[0] else None))
            y = _combine(part, 1, (yield))
            for row, cols, sign, gc, old in outs:
                v = _combine(old, sign, y)
                if gc is not None:
                    put(lay["b"] + row, cols, v * _cat([gc, gc], 1))
                else:
                    put(lay["acc"] + row, cols, v)

        def down_rest(kk, r):
            row = _T + 16 * r
            old = get(lay["acc"] + row, _cols(0)) if kk else None
            if kk < nk - 1:
                return put(lay["acc"] + row, _cols(0),
                           _combine(old, 1, (yield)))
            gc = gate_rows(16 * r)
            put(lay["b"] + row, _cols(0), _combine(old, 1, (yield)) * gc)

        waves = []
        for n in range(0, pairs, 2):
            bases = [wlay["gu"] + (n + j) * 4 * _T for j in range(2)]
            for i in range(7):
                row, col = _operand(lay["x"], i, _HT // 2)
                for j in range(2):
                    wrow, wcol = _operand(bases[j], i, _T)
                    waves.append((span(row, 4, _cols(col, 2)),
                                  weight(wrow, _T, _cols(wcol, 2)),
                                  functools.partial(gate_up, j, i)))
            row, col = _operand(lay["x"], 7, _HT // 2)
            for c in range(2):
                waves.append((
                    [[(row + 8 * (r // 2), _cols(col + r % 2))]
                     for r in range(8)],
                    lambda bases=bases, c=c: _cat(
                        (weight(base + 3 * _T + _HT * b, _HT, _cols(2 + c))()
                         for b in range(2) for base in bases), 1),
                    functools.partial(hidden, n + c)))
        for n in range(5):
            waves.append((
                span(lay["o"], 8, _cols(0, 4)),
                weight(wlay["o"] + 2 * _T * (n // 4), 2 * _T, _cols(n % 4)),
                functools.partial(project_out, n)))
        row = wlay["o"] + 2 * _T
        waves.append((
            span(lay["o"] + _HT, 8, _cols(0)),
            lambda row=row: _cat([weight(row, _HT, _cols(1, 3))(),
                                  weight(row + _HT, _HT, _cols(1))()], 1),
            functools.partial(emit, 0, 4)))
        waves.append((span(lay["o"] + _HT, 8, _cols(0)),
                      weight(row + _HT, _HT, _cols(2)),
                      functools.partial(emit, 4, 1)))
        single_tile = len(waves) - 1
        for i in range(7):
            if i < 2 * nk and i % 2 == 0:
                kk = i // 2
                row = wlay["down"] + (4 * kk + 3) * _T
                pieces = [[h_operand(2 * kk, m) for m in pair]
                          for pair in ((2, 7), (8, 3))]
                waves.append((
                    [[(r0 + 8 * (r % 4), _cols(c0, 2))
                      for r0, c0 in pieces[r // 4]] for r in range(8)],
                    lambda row=row: _cat((weight(row, _T, _cols(2 + half))()
                                          for half in range(2)), 0),
                    functools.partial(down_rest, kk)))
            for kk in range(nk):
                row, col = h_operand(2 * kk, i)
                wrow, wcol = _operand(wlay["down"] + kk * 4 * _T, i, _T)
                waves.append((span(row, 4, _cols(col, 2)),
                              weight(wrow, _T, _cols(wcol, 2)),
                              functools.partial(down, i, kk)))

        def stage_o(n):
            o = o_tile(n * _T, (n + 1) * _T)
            for r in range(0, _T, 32):
                live["now"] = (-1,)
                store(lay["o"] + _HT * (n // 4) + r // 2, _cols(n % 4),
                      _pack(o[r:r + 32]))
                yield

        def wave_load(w, r):
            live["now"] = (w, 0, r)
            live["lhs", w, r] = _cat(
                (load(row, 8, cols) for row, cols in waves[w][0][r]), 1)

        def wave(w):
            lhs = _unpack(_cat((live.pop(("lhs", w, r))
                                for r in range(len(waves[w][0]))), 0))
            rhs = waves[w][1]()
            if w == single_tile:
                live["y", w] = _cat(
                    (_dot(lhs[r:r + 32], rhs) for r in range(0, _T, 32)), 0)
            else:
                live["y", w] = _dot(lhs, rhs)

        def wave_fetch(w, r):
            live["now"] = (w, 1, r)
            live["end", w, r] = waves[w][2](r)
            next(live["end", w, r])

        def wave_done(w, r):
            live["now"] = (w, 2, r)
            try:
                live.pop(("end", w, r)).send(live["y", w][16 * r:16 * r + 16])
            except StopIteration:
                pass

        slots = _STEPS * nt
        cost = [32 if w == single_tile else 16 * len(waves[w][0])
                for w in range(len(waves))]
        host = []
        for w in range(len(waves)):
            share = (sum(cost[:w]) + cost[w] / 2) / sum(cost)
            host.append(max(int(share * (slots + _LAG)),
                            host[-1] + 1 if host else 0))
        host = [min(s, slots + _LAG - len(host) + w)
                for w, s in enumerate(host)]
        time = o_time = 0
        done, busy = {}, []
        for n in range(5):
            stores = stage_o(n)
            for m in range(4):
                line.at(400 + 250 * n + 32 * m, next, stores)
        stores = stage_gate()
        for m in range(8):
            line.at(1650 + 16 * m, next, stores)
        for r in range(0, _HT, 16):
            for c in range(2):
                x = 2500 + 90 * r + 700 * c
                line.at(x, stage_x, following, r, c)
                busy.append((x, 25))
        for s in range(slots + _LAG):
            if s < slots:
                u, c = divmod(s, nt)
                line.load_at(time - 20, q_load, u, c)
                for i, g in enumerate(chunks[c]):
                    line.load_at(time - 5, k_load, u, g)
                    done[u, g] = time + _SCORE_LATENCY + _phase(2, time)
                    line.at(done[u, g], p_store, u, c, i)
                    time += 16
                line.at(time, qk, u, c)
            if s in host:
                w = host.index(s)
                n = len(waves[w][0])
                for r in range(n):
                    line.load_at(time + 10, wave_load, w, r)
                    time += cost[w] // n
                    end = time - 16 + _WAVE_LATENCY + _phase(3, time)
                    line.load_at(end - 14, wave_fetch, w, r)
                    line.at(end, wave_done, w, r)
                    if waves[w][2].func is hidden:
                        busy.append((end - 14, 10))
                line.at(time, wave, w)
            if s >= _LAG:
                u, c = divmod(s - _LAG, nt)
                for i in range(4):
                    line.load_at(time - 88 + 22 * i, p_load, u, c, 3 - i)
                time += 24
                line.at(time, pv, u, c)
                o_time = max(time + _PV_LATENCY + _phase(4, time),
                             o_time + 14 + _BATCH)
                for r in (0, 8, 16):
                    if c:
                        line.load_at(o_time + r // 2 - 18, o_fetch, u, c, r)
                    line.at(o_time + r // 2 - 8, o_done, u, c, r)
                if c == nt - 1:
                    busy.append((time + 130, 10))
                if s >= slots - 1:
                    busy.append((time - 20, 40))
        rate = (sum(n for _, n in busy) + 80 * len(stages)) / (time + 100)
        when, used = [], 0
        busy.sort(reverse=True)
        while len(when) < len(stages):
            x = 55 + (used + 80) / rate
            if busy and busy[-1][0] <= x:
                used += busy.pop()[1]
            else:
                when.append(x + _phase(1, x))
                used += 80
        last = {}
        for (slot, u, e, i), x in zip(stages, when):
            line.load_at(x - 1, sums_fetch, slot, u, e, i,
                         after=last.get(slot, -1e9))
            line.at(x, scores, slot, u, e, i)
            last[slot] = x + 0.01
            done[u, e] = done[u, e + 1] = x
        for u in range(_STEPS):
            pv_order[u] = sorted(range(nt), key=lambda c, u=u: max(
                done.get((u, g), -1) for g in range(8 * c, 8 * c + 8)))
        line.run()

        @pl.when(t > 0)
        def _():
            out_copy(t - 1).start()

        @pl.when(t == 0)
        def _():
            wo_copy.wait()
            prepare_out(lambda r, c: _pack(wo_v[r, c]))

        return carry

    @pl.when(fast_ok)
    def _():
        lax.fori_loop(0, nt, fast_tile, None)
        row = lay["b"]
        b = pltpu.bitcast(_cat(
            [mem[row:row + _T, :], mem[row + _T:row + 2 * _T, _cols(0)]], 1),
            _F32)
        a = _dot(o_tile(0, dm).astype(_BF16), wo_v[...])
        out_v[seq - _T:seq, :] = (a + b).astype(out_v.dtype)
        out_copy(nt - 1).start()

    def safe_tile(t, carry):
        def head_pair(i, carry):
            outs = []
            for odd in range(2):
                j = 2 * (i & 1) + odd
                k = mem[lay["k"]:lay["k"] + seq // 2,
                        pl.ds(_al(j * _T, _T), _T)]
                s = _dot(_unpack(k)[:, :32], q_window(t, i >> 1, j))
                p = jnp.exp2(s - jnp.max(s, axis=0, keepdims=True))
                outs.append(normalise(_dot(vt_v[odd], p.astype(_BF16)), odd,
                                      t))
            mid = low_rows_from(outs[0][16:24], outs[1][0:8])
            ot_v[pl.ds(_al(2 * dh * i, 8), 2 * dh), :] = _cat(
                [outs[0][0:16], mid, outs[1][8:24]], 0)
            return carry

        lax.fori_loop(0, 4, head_pair, None)
        rows = pl.ds(_al(t * _T, _T), _T)
        xb = x_v[rows, :]
        h = jnp.maximum(_dot(xb, wgu_v[0]), 0.0) * _dot(xb, wgu_v[1])
        b = _dot(h.astype(_BF16), wd_v[...])
        a = _dot(o_tile(0, dm).astype(_BF16), wo_v[...])
        gc = _cat([one_minus_gate(t)] * (dm // _T), 1)
        out_v[rows, :] = (a + gc * b).astype(out_v.dtype)
        out_copy(t).start()
        return carry

    @pl.when(jnp.logical_not(fast_ok))
    def _():
        wo_copy.wait()
        lax.fori_loop(0, nt, safe_tile, None)

    for t in range(nt):
        out_copy(t).wait()


@jax.jit
def pallas_gated_mix__grouped_kv_mqa__glu_gated_reglu__prompt_kernel(
    A_x: jax.Array,
    A_wq: jax.Array,
    A_wk: jax.Array,
    A_wv: jax.Array,
    A_wo: jax.Array,
    B_x: jax.Array,
    B_W_gate: jax.Array,
    B_W_up: jax.Array,
    B_W_down: jax.Array,
    gate_w: jax.Array,
):
    del B_x
    batch, seq, dm = A_x.shape
    ff = B_W_gate.shape[1]
    assert (batch, seq, dm, ff) == (1, 4 * _PB, 5 * _T, 12 * _T)
    dh = dm // _H
    vmem = pltpu.VMEM
    ins = (A_x.reshape(seq, dm), A_wq, A_wk.T, A_wv.T, A_wo, B_W_gate, B_W_up,
           B_W_down, gate_w)
    out = pl.pallas_call(
        _kernel,
        out_shape=jax.ShapeDtypeStruct((seq, dm), A_x.dtype),
        in_specs=[pl.BlockSpec(memory_space=pl.ANY)] * len(ins),
        out_specs=pl.BlockSpec(memory_space=pl.ANY),
        scratch_shapes=[
            vmem((seq, dm), _BF16),
            vmem((dm, dm), _BF16),
            vmem((dm, dm), _BF16),
            vmem((ff, dm), _BF16),
            vmem((2, dm, ff), _BF16),
            vmem((seq, dm), A_x.dtype),
            *[vmem((rows, 4 * _T), _U32) for _, rows in _layouts(seq, dm, ff)],
            vmem((seq // _T, dm // 8, 4 * _T), _U32),
            vmem((seq // _T, dm // 4, 8 * _T), _F32),
            *[vmem((2 * n, 16 * dh, 4 * _T), _F32)
              for n in _TABLES],
            vmem((3, 24, seq), _F32),
            vmem((8, seq), _F32),
            vmem((dm // 4, 4 * _T), _F32),
            vmem((dh, dm), _BF16),
            vmem((dh, dm), _BF16),
            vmem((dm,), _BF16),
            pltpu.SMEM((_ZEROS,), jnp.int32),
            pltpu.SemaphoreType.DMA((8,)),
            pltpu.SemaphoreType.DMA((seq // _PB,)),
            pltpu.SemaphoreType.DMA,
        ],
        compiler_params=pltpu.CompilerParams(
            vmem_limit_bytes=100 * 1024 * 1024),
        name="gated_mix_mqa_reglu",
    )(*ins)
    return out.reshape(batch, seq, dm)
```
